```python
import os as _os
_os.environ.setdefault("JAX_PLATFORMS", "cpu")
import jax
import jax.numpy as jnp

def _softmax(x, axis=-1):
    return jax.nn.softmax(x, axis=axis)
def _gelu(x):
    return jax.nn.gelu(x, approximate=True)
def _silu(x):
    return jax.nn.silu(x)
def _sigmoid(x):
    return jax.nn.sigmoid(x)
def _layernorm(x, axis=-1, eps=1e-5):
    m = jnp.mean(x, axis=axis, keepdims=True)
    v = jnp.var(x, axis=axis, keepdims=True)
    return (x - m) / jnp.sqrt(v + eps)
def _scatter_add(tgt, idx, src, axis=0):
    return tgt.at[idx].add(src)
def _segment_sum(src, seg, n):
    return jax.ops.segment_sum(src, seg, n)
class _Rng:
    def __init__(self, key):
        self._k = key
    def _next(self):
        self._k, sub = jax.random.split(self._k)
        return sub
    def normal(self, shape):
        return jax.random.normal(self._next(), shape, dtype=jnp.bfloat16)
    def randint(self, lo, hi, shape):
        return jax.random.randint(self._next(), shape, lo, hi, dtype=jnp.int32)
    def uniform(self, shape, lo=0.0, hi=1.0):
        return jax.random.uniform(self._next(), shape, jnp.bfloat16, lo, hi)
    def permutation(self, n):
        return jax.random.permutation(self._next(), n)


kernel_name = 'gated_mix__ssm_conv_s5__glu_gated_geglu__prompt'

def setup_inputs():
    _rng = _Rng(jax.random.key(int.from_bytes(__import__("os").urandom(4), "little")))
    _w = (lambda a: (lambda t: t.astype(jnp.bfloat16) if jnp.issubdtype(t.dtype, jnp.floating) else t)(jnp.asarray(a)))
    def _A_setup():
        B, S, D = 1, 2048, 1024
        P = D
        Lambda_re = -0.5 * jnp.exp((lambda *s: _rng.normal(s) * 0.4)(P))
        Lambda_im = (lambda *s: _rng.normal(s) * 0.4)(P) * 1.0
        B_re = (lambda *s: _rng.normal(s) * 0.4)(P, D) * (D ** -0.5)
        B_im = (lambda *s: _rng.normal(s) * 0.4)(P, D) * (D ** -0.5)
        C_re = (lambda *s: _rng.normal(s) * 0.4)(D, P) * (P ** -0.5)
        C_im = (lambda *s: _rng.normal(s) * 0.4)(D, P) * (P ** -0.5)
        log_dt = (lambda *s: _rng.normal(s) * 0.4)(P) * 0.3 - 2.0
        Dskip = (lambda *s: _rng.normal(s) * 0.4)(D)
        return {
            "x": _w((lambda *s: _rng.normal(s) * 0.05)(B, S, D)),
            "Lambda_re": _w(Lambda_re),
            "Lambda_im": _w(Lambda_im),
            "B_re": _w(B_re),
            "B_im": _w(B_im),
            "C_re": _w(C_re),
            "C_im": _w(C_im),
            "log_dt": _w(log_dt),
            "Dskip": _w(Dskip),
        }
    _A_in = _A_setup()

    def _B_setup():
        B, S, Dm, Df = 1, 2048, 1024, 3584
        return {
            "x": _w((lambda *s: _rng.normal(s) * 0.05)(B, S, Dm)),
            "w_gate": _w((lambda *s: _rng.normal(s) * 1.6)(Dm, Df) * (Dm ** -0.5)),
            "w_up": _w((lambda *s: _rng.normal(s) * 1.6)(Dm, Df) * (Dm ** -0.5)),
            "w_down": _w((lambda *s: _rng.normal(s) * 1.6)(Df, Dm) * (Df ** -0.5)),
        }
    _B_in = _B_setup()

    return {
        "A_x": _A_in["x"],
        "A_Lambda_re": _A_in["Lambda_re"],
        "A_Lambda_im": _A_in["Lambda_im"],
        "A_B_re": _A_in["B_re"],
        "A_B_im": _A_in["B_im"],
        "A_C_re": _A_in["C_re"],
        "A_C_im": _A_in["C_im"],
        "A_log_dt": _A_in["log_dt"],
        "A_Dskip": _A_in["Dskip"],
        "B_x": _B_in["x"],
        "B_w_gate": _B_in["w_gate"],
        "B_w_up": _B_in["w_up"],
        "B_w_down": _B_in["w_down"],
        "gate_w": _w((lambda *s: _rng.normal(s) * 0.05)(1024) * 16.0),
    }

def reference(A_x, A_Lambda_re, A_Lambda_im, A_B_re, A_B_im, A_C_re, A_C_im, A_log_dt, A_Dskip, B_x, B_w_gate, B_w_up, B_w_down, gate_w):
    def _A_ref(x, Lambda_re, Lambda_im, B_re, B_im, C_re, C_im, log_dt, Dskip):
        Bsz, L, H = x.shape
        Lam = Lambda_re + 1j * Lambda_im
        Bmat = B_re + 1j * B_im
        Cmat = C_re + 1j * C_im
        dt = jnp.exp(log_dt)
        Lam_bar = jnp.exp(dt * Lam)
        B_bar = ((Lam_bar - 1.0) / Lam)[:, None] * Bmat
        Bu = jnp.einsum("bld,pd->blp", x + 0j, B_bar)
        h = jnp.zeros_like(Bu[:, 0, :])
        hs = []
        for t in range(L):
            h = Lam_bar[None, :] * h + Bu[:, t, :]
            hs.append(h)
        hseq = jnp.stack(hs, 1)
        y = 2.0 * jnp.einsum("blp,dp->bld", hseq, Cmat).real + x * Dskip[None, None, :]
        return y

    def _B_ref(x, w_gate, w_up, w_down):
        g = jnp.einsum("bsd,df->bsf", x, w_gate)
        u = jnp.einsum("bsd,df->bsf", x, w_up)
        h = _gelu(g) * u
        return jnp.einsum("bsf,fd->bsd", h, w_down)

    x = A_x
    g = _sigmoid((x * gate_w).sum(-1, keepdims=True))
    a = _A_ref(x, A_Lambda_re, A_Lambda_im, A_B_re, A_B_im, A_C_re, A_C_im, A_log_dt, A_Dskip)
    b = _B_ref(x, B_w_gate, B_w_up, B_w_down)
    return g * a + (1 - g) * b
```

```python
import functools

import jax
import jax.numpy as jnp
import jax.experimental.pallas as pl
import jax.experimental.pallas.tpu as pltpu

T_BLK = 512
F_BLK = 512
NSEG = 8


def _nt_dot(a, b):
    return jax.lax.dot_general(a, b, (((1,), (1,)), ((), ())),
                               preferred_element_type=jnp.float32)


def _kernel(x_ref, lre_ref, lim_ref, ldt_ref, dsk_ref, gw_ref,
            bre_ref, bim_ref, cre_ref, cim_ref, wg_ref, wu_ref, wd_ref,
            o_ref,
            bcat_ref, ccat_ref, v_ref, coef_ref, carry_ref,
            *, P, D, F, T):
    i = pl.program_id(0)
    S = T // NSEG

    @pl.when(i == 0)
    def _init():
        lre = lre_ref[...].astype(jnp.float32)
        lim = lim_ref[...].astype(jnp.float32)
        dt = jnp.exp(ldt_ref[...].astype(jnp.float32))
        dt = dt.astype(jnp.bfloat16).astype(jnp.float32)
        zr = dt * lre
        zi = dt * lim
        mag = jnp.exp(zr)
        a_re = mag * jnp.cos(zi)
        a_im = mag * jnp.sin(zi)
        nr = a_re - 1.0
        ni = a_im
        den = lre * lre + lim * lim
        m_re = (nr * lre + ni * lim) / den
        m_im = (ni * lre - nr * lim) / den
        p_re, p_im = a_re, a_im
        for _ in range(S.bit_length() - 1):
            p_re, p_im = p_re * p_re - p_im * p_im, 2.0 * p_re * p_im
        coef_ref[0:1, :] = a_re
        coef_ref[1:2, :] = a_im
        coef_ref[2:3, :] = p_re
        coef_ref[3:4, :] = p_im
        coef_ref[4:8, :] = jnp.zeros((4, P), jnp.float32)
        m_re_c = jnp.transpose(jnp.broadcast_to(m_re, (128, P)))[:, 0:1]
        m_im_c = jnp.transpose(jnp.broadcast_to(m_im, (128, P)))[:, 0:1]
        bre = bre_ref[...].astype(jnp.float32)
        bim = bim_ref[...].astype(jnp.float32)
        bcat_ref[0:P, :] = (m_re_c * bre - m_im_c * bim).astype(jnp.bfloat16)
        bcat_ref[P:2 * P, :] = (m_re_c * bim + m_im_c * bre).astype(jnp.bfloat16)
        ccat_ref[:, 0:P] = (2.0 * cre_ref[...].astype(jnp.float32)).astype(jnp.bfloat16)
        ccat_ref[:, P:2 * P] = (-2.0 * cim_ref[...].astype(jnp.float32)).astype(jnp.bfloat16)
        carry_ref[...] = jnp.zeros(carry_ref.shape, jnp.float32)

    x = x_ref[...]

    NT = 2 * P // 128
    HT = P // 128
    v = _nt_dot(x, bcat_ref[...])
    for k in range(NT):
        v_ref[k] = v[:, k * 128:(k + 1) * 128]

    KC = 4
    for c in range(HT // KC):
        ks = list(range(c * KC, (c + 1) * KC))
        a_re = [jnp.broadcast_to(coef_ref[0:1, k * 128:(k + 1) * 128], (NSEG, 128)) for k in ks]
        a_im = [jnp.broadcast_to(coef_ref[1:2, k * 128:(k + 1) * 128], (NSEG, 128)) for k in ks]

        def step(hh, j, store):
            out = []
            for n, k in enumerate(ks):
                h_re, h_im = hh[2 * n], hh[2 * n + 1]
                vr = v_ref[k, pl.ds(j, NSEG, stride=S), :]
                vi = v_ref[HT + k, pl.ds(j, NSEG, stride=S), :]
                n_re = a_re[n] * h_re - a_im[n] * h_im + vr
                n_im = a_re[n] * h_im + a_im[n] * h_re + vi
                if store:
                    v_ref[k, pl.ds(j, NSEG, stride=S), :] = n_re
                    v_ref[HT + k, pl.ds(j, NSEG, stride=S), :] = n_im
                out += [n_re, n_im]
            return tuple(out)

        z = jnp.zeros((NSEG, 128), jnp.float32)
        e = jax.lax.fori_loop(0, S, lambda j, hh: step(hh, j, False), (z,) * (2 * KC), unroll=8)

        init = []
        for n, k in enumerate(ks):
            sl = slice(k * 128, (k + 1) * 128)
            e_re, e_im = e[2 * n], e[2 * n + 1]
            p_re = coef_ref[2:3, sl]
            p_im = coef_ref[3:4, sl]
            c_re = carry_ref[0:1, sl]
            c_im = carry_ref[1:2, sl]
            rows_re, rows_im = [], []
            for r in range(NSEG):
                rows_re.append(c_re)
                rows_im.append(c_im)
                n_re = e_re[r:r + 1] + p_re * c_re - p_im * c_im
                n_im = e_im[r:r + 1] + p_re * c_im + p_im * c_re
                c_re, c_im = n_re, n_im
            carry_ref[0:1, sl] = c_re
            carry_ref[1:2, sl] = c_im
            init += [jnp.concatenate(rows_re, axis=0), jnp.concatenate(rows_im, axis=0)]

        jax.lax.fori_loop(0, S, lambda j, hh: step(hh, j, True), tuple(init), unroll=8)

    h = jnp.concatenate([v_ref[k].astype(jnp.bfloat16) for k in range(NT)], axis=1)
    y = _nt_dot(h, ccat_ref[...])

    acc = jnp.zeros((T, D), jnp.float32)
    for f in range(F // F_BLK):
        fl = f * F_BLK
        g = jnp.dot(x, wg_ref[:, fl:fl + F_BLK], preferred_element_type=jnp.float32)
        u = jnp.dot(x, wu_ref[:, fl:fl + F_BLK], preferred_element_type=jnp.float32)
        g = g.astype(jnp.bfloat16).astype(jnp.float32)
        u = u.astype(jnp.bfloat16).astype(jnp.float32)
        hm = (jax.nn.gelu(g, approximate=True) * u).astype(jnp.bfloat16)
        acc = acc + jnp.dot(hm, wd_ref[fl:fl + F_BLK, :], preferred_element_type=jnp.float32)
    b = acc.astype(jnp.bfloat16).astype(jnp.float32)

    xf = x.astype(jnp.float32)
    prod = (xf * gw_ref[...].astype(jnp.float32)).astype(jnp.bfloat16).astype(jnp.float32)
    s = jnp.sum(prod, axis=-1, keepdims=True).astype(jnp.bfloat16).astype(jnp.float32)
    gate = jax.nn.sigmoid(s).astype(jnp.bfloat16).astype(jnp.float32)
    skip = (xf * dsk_ref[...].astype(jnp.float32)).astype(jnp.bfloat16).astype(jnp.float32)
    a = y + skip
    omg = (1.0 - gate).astype(jnp.bfloat16).astype(jnp.float32)
    t2 = (omg * b).astype(jnp.bfloat16).astype(jnp.float32)
    o_ref[...] = gate * a + t2


@jax.jit
def pallas_gated_mix__ssm_conv_s5__glu_gated_geglu__prompt_kernel(
    A_x: jax.Array,
    A_Lambda_re: jax.Array,
    A_Lambda_im: jax.Array,
    A_B_re: jax.Array,
    A_B_im: jax.Array,
    A_C_re: jax.Array,
    A_C_im: jax.Array,
    A_log_dt: jax.Array,
    A_Dskip: jax.Array,
    B_x: jax.Array,
    B_w_gate: jax.Array,
    B_w_up: jax.Array,
    B_w_down: jax.Array,
    gate_w: jax.Array,
):
    Bsz, L, D = A_x.shape
    P = A_Lambda_re.shape[0]
    F = B_w_gate.shape[1]
    assert Bsz == 1
    T = T_BLK
    x2 = A_x.reshape(L, D)
    row = lambda a: a.reshape(1, -1)

    const = lambda shape: pl.BlockSpec(shape, lambda i: (0, 0), pipeline_mode=pl.Buffered(1))
    in_specs = [
        pl.BlockSpec((T, D), lambda i: (i, 0)),
        const((1, P)), const((1, P)), const((1, P)), const((1, D)), const((1, D)),
        const((P, D)), const((P, D)), const((D, P)), const((D, P)),
        const((D, F)), const((D, F)), const((F, D)),
    ]
    out = pl.pallas_call(
        functools.partial(_kernel, P=P, D=D, F=F, T=T),
        grid=(L // T,),
        in_specs=in_specs,
        out_specs=pl.BlockSpec((T, D), lambda i: (i, 0)),
        out_shape=jax.ShapeDtypeStruct((L, D), jnp.float32),
        scratch_shapes=[
            pltpu.VMEM((2 * P, D), jnp.bfloat16),
            pltpu.VMEM((D, 2 * P), jnp.bfloat16),
            pltpu.VMEM((2 * P // 128, T, 128), jnp.float32),
            pltpu.VMEM((8, P), jnp.float32),
            pltpu.VMEM((8, P), jnp.float32),
        ],
        compiler_params=pltpu.CompilerParams(
            dimension_semantics=("arbitrary",),
            vmem_limit_bytes=100 * 1024 * 1024,
        ),
    )(x2, row(A_Lambda_re), row(A_Lambda_im), row(A_log_dt), row(A_Dskip), row(gate_w),
      A_B_re, A_B_im, A_C_re, A_C_im, B_w_gate, B_w_up, B_w_down)
    return out.reshape(Bsz, L, D)
```

```python
import functools

import jax
import jax.numpy as jnp
import jax.experimental.pallas as pl
import jax.experimental.pallas.tpu as pltpu

T_BLK = 512
F_BLK = 512
SCOPES = False


class _NoScope:
    def __enter__(self):
        return self

    def __exit__(self, *a):
        return False


def _scope(name):
    return jax.named_scope(name) if SCOPES else _NoScope()


def _nt_dot(a, b):
    return jax.lax.dot_general(a, b, (((1,), (1,)), ((), ())),
                               preferred_element_type=jnp.float32)


def _cmul(ar, ai, br, bi):
    return ar * br - ai * bi, ar * bi + ai * br


def _kernel(x_ref, lre_ref, lim_ref, ldt_ref, dsk_ref, gw_ref,
            bre_hbm, bim_hbm, cre_hbm, cim_hbm, wg_hbm, wu_hbm, wd_hbm,
            o_ref,
            bre_v, bim_v, cre_v, cim_v, wg_v, wu_v, wd_v,
            bcat_ref, ccat_ref, v_ref, h_ref, tab_ref, carry_ref, mcol_ref, acc_ref, sems,
            *, P, D, F, T):
    i = pl.program_id(0)
    NF = F // F_BLK
    HT = P // 128
    first = i == 0

    def g_copies(f):
        fs = pl.ds(pl.multiple_of(f * F_BLK, F_BLK), F_BLK)
        return [
            pltpu.make_async_copy(wg_hbm.at[:, fs], wg_v.at[:, fs], sems.at[4 + 3 * f]),
            pltpu.make_async_copy(wu_hbm.at[:, fs], wu_v.at[:, fs], sems.at[5 + 3 * f]),
            pltpu.make_async_copy(wd_hbm.at[fs, :], wd_v.at[fs, :], sems.at[6 + 3 * f]),
        ]

    def b_copies():
        return [pltpu.make_async_copy(bre_hbm, bre_v, sems.at[0]),
                pltpu.make_async_copy(bim_hbm, bim_v, sems.at[1])]

    def c_copies():
        return [pltpu.make_async_copy(cre_hbm, cre_v, sems.at[2]),
                pltpu.make_async_copy(cim_hbm, cim_v, sems.at[3])]

    @pl.when(first)
    def _():
        for cp in g_copies(0) + g_copies(1):
            cp.start()
        with _scope('init'):
            lre = lre_ref[...].astype(jnp.float32)
            lim = lim_ref[...].astype(jnp.float32)
            dt = jnp.exp(ldt_ref[...].astype(jnp.float32))
            dt = dt.astype(jnp.bfloat16).astype(jnp.float32)
            mag = jnp.exp(dt * lre)
            a_re = mag * jnp.cos(dt * lim)
            a_im = mag * jnp.sin(dt * lim)
            nr = a_re - 1.0
            ni = a_im
            den = lre * lre + lim * lim
            m_re = (nr * lre + ni * lim) / den
            m_im = (ni * lre - nr * lim) / den
            pw = [(a_re, a_im)]
            for _ in range(7):
                pw.append(_cmul(pw[-1][0], pw[-1][1], a_re, a_im))
            rid = jax.lax.broadcasted_iota(jnp.int32, (8, P), 0)
            for n, k in enumerate((1, 2, 4)):
                tab_ref[2 * n] = jnp.where(rid >= k, pw[k - 1][0], 0.0)
                tab_ref[2 * n + 1] = jnp.where(rid >= k, pw[k - 1][1], 0.0)
            tab_ref[6] = jnp.concatenate([p[0] for p in pw], axis=0)
            tab_ref[7] = jnp.concatenate([p[1] for p in pw], axis=0)
            carry_ref[...] = jnp.zeros(carry_ref.shape, jnp.float32)
            mcol_ref[0] = jnp.transpose(jnp.broadcast_to(m_re, (128, P)))
            mcol_ref[1] = jnp.transpose(jnp.broadcast_to(m_im, (128, P)))

    x = x_ref[...]

    acc_ref[...] = jnp.zeros(acc_ref.shape, jnp.float32)

    def geglu_step(f, carry):
        @pl.when(first)
        def _():
            @pl.when(f + 2 < NF)
            def _():
                for cp in g_copies(f + 2):
                    cp.start()

            @pl.when(f == 1)
            def _():
                for cp in b_copies():
                    cp.start()

            @pl.when(f == 2)
            def _():
                for cp in c_copies():
                    cp.start()

            for cp in g_copies(f):
                cp.wait()

        fs = pl.ds(pl.multiple_of(f * F_BLK, F_BLK), F_BLK)
        xx = x_ref[...]
        g = jnp.dot(xx, wg_v[:, fs], preferred_element_type=jnp.float32)
        u = jnp.dot(xx, wu_v[:, fs], preferred_element_type=jnp.float32)
        g = g.astype(jnp.bfloat16).astype(jnp.float32)
        u = u.astype(jnp.bfloat16).astype(jnp.float32)
        hm = (jax.nn.gelu(g, approximate=True) * u).astype(jnp.bfloat16)
        acc_ref[...] += jnp.dot(hm, wd_v[fs, :], preferred_element_type=jnp.float32)
        return carry

    with _scope('geglu'):
        jax.lax.fori_loop(0, NF, geglu_step, 0)

    @pl.when(first)
    def _():
        for cp in b_copies():
            cp.wait()
        with _scope('bcat'):
            m_re_c = mcol_ref[0][:, 0:1]
            m_im_c = mcol_ref[1][:, 0:1]
            bre = bre_v[...].astype(jnp.float32)
            bim = bim_v[...].astype(jnp.float32)
            bcat_ref[0:P, :] = (m_re_c * bre - m_im_c * bim).astype(jnp.bfloat16)
            bcat_ref[P:2 * P, :] = (m_re_c * bim + m_im_c * bre).astype(jnp.bfloat16)
        for cp in c_copies():
            cp.wait()
        with _scope('ccat'):
            ccat_ref[:, 0:P] = (2.0 * cre_v[...].astype(jnp.float32)).astype(jnp.bfloat16)
            ccat_ref[:, P:2 * P] = (-2.0 * cim_v[...].astype(jnp.float32)).astype(jnp.bfloat16)

    with _scope('bmm'):
        v_ref[...] = _nt_dot(x, bcat_ref[...])

    with _scope('scan'):
        for k in range(HT):
            sl = slice(k * 128, (k + 1) * 128)
            si = slice(P + k * 128, P + (k + 1) * 128)
            tabs = [tab_ref[n, :, sl] for n in range(8)]
            c_re = carry_ref[0:1, sl]
            c_im = carry_ref[1:2, sl]
            for q in range(T // 16):
                outs = []
                for half in range(2):
                    r0 = q * 16 + half * 8
                    h_re = v_ref[r0:r0 + 8, sl]
                    h_im = v_ref[r0:r0 + 8, si]
                    for n, sh in enumerate((1, 2, 4)):
                        r_re = pltpu.roll(h_re, sh, 0)
                        r_im = pltpu.roll(h_im, sh, 0)
                        d_re, d_im = _cmul(tabs[2 * n], tabs[2 * n + 1], r_re, r_im)
                        h_re = h_re + d_re
                        h_im = h_im + d_im
                    cb_re = jnp.broadcast_to(c_re, (8, 128))
                    cb_im = jnp.broadcast_to(c_im, (8, 128))
                    d_re, d_im = _cmul(tabs[6], tabs[7], cb_re, cb_im)
                    h_re = h_re + d_re
                    h_im = h_im + d_im
                    c_re = h_re[7:8]
                    c_im = h_im[7:8]
                    outs.append((h_re, h_im))
                h_ref[q * 16:(q + 1) * 16, sl] = jnp.concatenate(
                    [outs[0][0], outs[1][0]], axis=0).astype(jnp.bfloat16)
                h_ref[q * 16:(q + 1) * 16, si] = jnp.concatenate(
                    [outs[0][1], outs[1][1]], axis=0).astype(jnp.bfloat16)
            carry_ref[0:1, sl] = c_re
            carry_ref[1:2, sl] = c_im

    with _scope('cmm'):
        y = _nt_dot(h_ref[...], ccat_ref[...])

    with _scope('mix'):
        b = acc_ref[...].astype(jnp.bfloat16).astype(jnp.float32)
        xf = x.astype(jnp.float32)
        prod = (xf * gw_ref[...].astype(jnp.float32)).astype(jnp.bfloat16).astype(jnp.float32)
        s = jnp.sum(prod, axis=-1, keepdims=True).astype(jnp.bfloat16).astype(jnp.float32)
        gate = jax.nn.sigmoid(s).astype(jnp.bfloat16).astype(jnp.float32)
        skip = (xf * dsk_ref[...].astype(jnp.float32)).astype(jnp.bfloat16).astype(jnp.float32)
        a = y + skip
        omg = (1.0 - gate).astype(jnp.bfloat16).astype(jnp.float32)
        t2 = (omg * b).astype(jnp.bfloat16).astype(jnp.float32)
        o_ref[...] = gate * a + t2


@jax.jit
def pallas_gated_mix__ssm_conv_s5__glu_gated_geglu__prompt_kernel(
    A_x: jax.Array,
    A_Lambda_re: jax.Array,
    A_Lambda_im: jax.Array,
    A_B_re: jax.Array,
    A_B_im: jax.Array,
    A_C_re: jax.Array,
    A_C_im: jax.Array,
    A_log_dt: jax.Array,
    A_Dskip: jax.Array,
    B_x: jax.Array,
    B_w_gate: jax.Array,
    B_w_up: jax.Array,
    B_w_down: jax.Array,
    gate_w: jax.Array,
):
    Bsz, L, D = A_x.shape
    P = A_Lambda_re.shape[0]
    F = B_w_gate.shape[1]
    assert Bsz == 1
    T = T_BLK
    NF = F // F_BLK
    x2 = A_x.reshape(L, D)
    row = lambda a: a.reshape(1, -1)

    const = lambda shape: pl.BlockSpec(shape, lambda i: (0, 0))
    hbm = pl.BlockSpec(memory_space=pl.ANY)
    in_specs = [
        pl.BlockSpec((T, D), lambda i: (i, 0)),
        const((1, P)), const((1, P)), const((1, P)), const((1, D)), const((1, D)),
        hbm, hbm, hbm, hbm, hbm, hbm, hbm,
    ]
    bf = jnp.bfloat16
    out = pl.pallas_call(
        functools.partial(_kernel, P=P, D=D, F=F, T=T),
        grid=(L // T,),
        in_specs=in_specs,
        out_specs=pl.BlockSpec((T, D), lambda i: (i, 0)),
        out_shape=jax.ShapeDtypeStruct((L, D), jnp.float32),
        scratch_shapes=[
            pltpu.VMEM((P, D), bf), pltpu.VMEM((P, D), bf),
            pltpu.VMEM((D, P), bf), pltpu.VMEM((D, P), bf),
            pltpu.VMEM((D, F), bf), pltpu.VMEM((D, F), bf), pltpu.VMEM((F, D), bf),
            pltpu.VMEM((2 * P, D), bf),
            pltpu.VMEM((D, 2 * P), bf),
            pltpu.VMEM((T, 2 * P), jnp.float32),
            pltpu.VMEM((T, 2 * P), bf),
            pltpu.VMEM((8, 8, P), jnp.float32),
            pltpu.VMEM((8, P), jnp.float32),
            pltpu.VMEM((2, P, 128), jnp.float32),
            pltpu.VMEM((T, D), jnp.float32),
            pltpu.SemaphoreType.DMA((4 + 3 * NF,)),
        ],
        compiler_params=pltpu.CompilerParams(
            dimension_semantics=("arbitrary",),
            vmem_limit_bytes=100 * 1024 * 1024,
        ),
    )(x2, row(A_Lambda_re), row(A_Lambda_im), row(A_log_dt), row(A_Dskip), row(gate_w),
      A_B_re, A_B_im, A_C_re, A_C_im, B_w_gate, B_w_up, B_w_down)
    return out.reshape(Bsz, L, D)
```

```python
import functools

import jax
import jax.numpy as jnp
import jax.experimental.pallas as pl
import jax.experimental.pallas.tpu as pltpu

T_BLK = 512
F_BLK = 512
SCOPES = False


class _NoScope:
    def __enter__(self):
        return self

    def __exit__(self, *a):
        return False


def _scope(name):
    return jax.named_scope(name) if SCOPES else _NoScope()


def _nt_dot(a, b):
    return jax.lax.dot_general(a, b, (((1,), (1,)), ((), ())),
                               preferred_element_type=jnp.float32)


def _cmul(ar, ai, br, bi):
    return ar * br - ai * bi, ar * bi + ai * br


def _kernel(x_hbm, lre_ref, lim_ref, ldt_ref, dsk_ref, gw_ref,
            bre_hbm, bim_hbm, cre_hbm, cim_hbm, wg_hbm, wu_hbm, wd_hbm,
            o_hbm,
            wg_v, wu_v, wd_v,
            bcat_ref, ccat_ref, v_ref, h_ref, tab_ref, carry_ref, acc_ref, xbuf, obuf, sems, xsem, osem,
            *, P, D, F, T):
    i = pl.program_id(0)
    NF = F // F_BLK
    HT = P // 128
    first = i == 0
    nsteps = pl.num_programs(0)
    slot = i % 2
    NO = 4
    OC = D // NO

    def x_copy(step, sl):
        return pltpu.make_async_copy(x_hbm.at[pl.ds(pl.multiple_of(step * T, T), T), :], xbuf.at[sl], xsem.at[sl])

    def o_copy(step, n):
        return pltpu.make_async_copy(obuf.at[:, n * OC:(n + 1) * OC],
                                     o_hbm.at[pl.ds(pl.multiple_of(step * T, T), T), n * OC:(n + 1) * OC],
                                     osem.at[n])

    def g_copies(f):
        fs = pl.ds(pl.multiple_of(f * F_BLK, F_BLK), F_BLK)
        return [
            pltpu.make_async_copy(wg_hbm.at[:, fs], wg_v.at[:, fs], sems.at[4 + 3 * f]),
            pltpu.make_async_copy(wu_hbm.at[:, fs], wu_v.at[:, fs], sems.at[5 + 3 * f]),
            pltpu.make_async_copy(wd_hbm.at[fs, :], wd_v.at[fs, :], sems.at[6 + 3 * f]),
        ]

    def b_copies():
        return [pltpu.make_async_copy(bre_hbm, bcat_ref.at[0:P, :], sems.at[0]),
                pltpu.make_async_copy(bim_hbm, bcat_ref.at[P:2 * P, :], sems.at[1])]

    def c_copies():
        return [pltpu.make_async_copy(cre_hbm, ccat_ref.at[:, 0:P], sems.at[2]),
                pltpu.make_async_copy(cim_hbm, ccat_ref.at[:, P:2 * P], sems.at[3])]

    @pl.when(first)
    def _():
        x_copy(0, 0).start()
        for cp in g_copies(0):
            cp.start()
        with _scope('init'):
            lre = lre_ref[...].astype(jnp.float32).reshape(1, P)
            lim = lim_ref[...].astype(jnp.float32).reshape(1, P)
            dt = jnp.exp(ldt_ref[...].astype(jnp.float32).reshape(1, P))
            dt = dt.astype(jnp.bfloat16).astype(jnp.float32)
            mag = jnp.exp(dt * lre)
            a_re = mag * jnp.cos(dt * lim)
            a_im = mag * jnp.sin(dt * lim)
            nr = a_re - 1.0
            ni = a_im
            den = lre * lre + lim * lim
            m_re = (nr * lre + ni * lim) / den
            m_im = (ni * lre - nr * lim) / den
            pw = [(a_re, a_im)]
            for _ in range(7):
                pw.append(_cmul(pw[-1][0], pw[-1][1], a_re, a_im))
            rid = jax.lax.broadcasted_iota(jnp.int32, (8, P), 0)
            tabs = []
            for n, k in enumerate((1, 2, 4)):
                tabs.append(jnp.where(rid >= k, pw[k - 1][0], 0.0))
                tabs.append(jnp.where(rid >= k, pw[k - 1][1], 0.0))
            tabs.append(jnp.concatenate([p[0] for p in pw], axis=0))
            tabs.append(jnp.concatenate([p[1] for p in pw], axis=0))
            tabs.append(jnp.broadcast_to(m_re, (8, P)))
            tabs.append(jnp.broadcast_to(m_im, (8, P)))
            for k in range(HT):
                for n in range(10):
                    tab_ref[k, n] = tabs[n][:, k * 128:(k + 1) * 128]
            carry_ref[...] = jnp.zeros(carry_ref.shape, jnp.float32)

    acc_ref[...] = jnp.zeros(acc_ref.shape, jnp.float32)

    x_copy(i, slot).wait()
    x_ref = xbuf.at[slot]
    x = x_ref[...]

    def dma_ctl(f):
        @pl.when(first)
        def _():
            for cp in g_copies(f):
                cp.wait()

            @pl.when(f + 1 < NF)
            def _():
                for cp in g_copies(f + 1):
                    cp.start()

            @pl.when(f == 0)
            def _():
                for cp in b_copies():
                    cp.start()

            @pl.when(f == 2)
            def _():
                for cp in c_copies():
                    cp.start()

    def geglu(f):
        fs = pl.ds(pl.multiple_of(f * F_BLK, F_BLK), F_BLK)
        xx = x_ref[...]
        g = jnp.dot(xx, wg_v[:, fs], preferred_element_type=jnp.float32)
        u = jnp.dot(xx, wu_v[:, fs], preferred_element_type=jnp.float32)
        g = g.astype(jnp.bfloat16).astype(jnp.float32)
        u = u.astype(jnp.bfloat16).astype(jnp.float32)
        hm = (jax.nn.gelu(g, approximate=True) * u).astype(jnp.bfloat16)
        acc_ref[...] += jnp.dot(hm, wd_v[fs, :], preferred_element_type=jnp.float32)

    def scan_rows(k, q_lo, q_hi, st):
        tabs, c_re, c_im = st
        for q in range(q_lo, q_hi):
            outs = []
            for half in range(2):
                r0 = q * 16 + half * 8
                h_re, h_im = _cmul(tabs[8], tabs[9], v_ref[k, r0:r0 + 8, :], v_ref[HT + k, r0:r0 + 8, :])
                for n, sh in enumerate((1, 2, 4)):
                    r_re = pltpu.roll(h_re, sh, 0)
                    r_im = pltpu.roll(h_im, sh, 0)
                    d_re, d_im = _cmul(tabs[2 * n], tabs[2 * n + 1], r_re, r_im)
                    h_re = h_re + d_re
                    h_im = h_im + d_im
                cb_re = jnp.broadcast_to(c_re, (8, 128))
                cb_im = jnp.broadcast_to(c_im, (8, 128))
                d_re, d_im = _cmul(tabs[6], tabs[7], cb_re, cb_im)
                h_re = h_re + d_re
                h_im = h_im + d_im
                c_re = h_re[7:8]
                c_im = h_im[7:8]
                outs.append((h_re, h_im))
            h_ref[k, q * 16:(q + 1) * 16, :] = (2.0 * jnp.concatenate(
                [outs[0][0], outs[1][0]], axis=0)).astype(jnp.bfloat16)
            h_ref[HT + k, q * 16:(q + 1) * 16, :] = (-2.0 * jnp.concatenate(
                [outs[0][1], outs[1][1]], axis=0)).astype(jnp.bfloat16)
        return tabs, c_re, c_im

    NA = 3
    TPI = HT // (NF - NA)
    NPIECE = 16
    QPP = TPI * (T // 16) // NPIECE

    def loop_a(f, carry):
        dma_ctl(f)
        geglu(f)
        return carry

    def loop_b(f, carry):
        dma_ctl(f)
        k0 = (f - NA) * TPI
        state = [None]

        def scan_piece(p):
            t, qq = divmod(p * QPP, T // 16)
            k = k0 + t
            if qq == 0:
                state[0] = ([tab_ref[k, n] for n in range(10)],
                            carry_ref[k, 0:1, :], carry_ref[k, 1:2, :])
            state[0] = scan_rows(k, qq, qq + QPP, state[0])
            if qq + QPP == T // 16:
                carry_ref[k, 0:1, :] = state[0][1]
                carry_ref[k, 1:2, :] = state[0][2]

        def tie(dep):
            tabs, c_re, c_im = state[0]
            c_re = jnp.where(dep[0:1, 0:128] > jnp.inf, dep[0:1, 0:128], c_re)
            state[0] = (tabs, c_re, c_im)

        xx = x_ref[...]
        p = 0
        hms = []
        dep = None
        for n in range(4):
            fs = pl.ds(pl.multiple_of(f * F_BLK + n * 128, 128), 128)
            scan_piece(p); p += 1
            g = jnp.dot(xx, wg_v[:, fs], preferred_element_type=jnp.float32)
            tie(g)
            scan_piece(p); p += 1
            u = jnp.dot(xx, wu_v[:, fs], preferred_element_type=jnp.float32)
            if p % (NPIECE // TPI) != 0:
                tie(u)
            g = g.astype(jnp.bfloat16).astype(jnp.float32)
            u = u.astype(jnp.bfloat16).astype(jnp.float32)
            hms.append((jax.nn.gelu(g, approximate=True) * u).astype(jnp.bfloat16))
        hm = jnp.concatenate(hms, axis=1)
        fs = pl.ds(pl.multiple_of(f * F_BLK, F_BLK), F_BLK)
        for n in range(8):
            scan_piece(p); p += 1
            cs = slice(n * 128, (n + 1) * 128)
            d = jnp.dot(hm, wd_v[fs, cs], preferred_element_type=jnp.float32)
            if p < NPIECE:
                tie(d)
            acc_ref[:, cs] += d
        return carry

    with _scope('loopA'):
        jax.lax.fori_loop(0, NA, loop_a, 0)

    @pl.when(first)
    def _():
        for cp in b_copies():
            cp.wait()

    with _scope('bmm'):
        v = _nt_dot(x, bcat_ref[...])
        for k in range(2 * HT):
            v_ref[k] = v[:, k * 128:(k + 1) * 128]

    with _scope('loopB'):
        jax.lax.fori_loop(NA, NF, loop_b, 0)

    @pl.when(first)
    def _():
        for cp in c_copies():
            cp.wait()

    @pl.when(i + 1 < nsteps)
    def _():
        x_copy(i + 1, 1 - slot).start()

    h = jnp.concatenate([h_ref[k] for k in range(2 * HT)], axis=1)

    with _scope('mix'):
        xf = x.astype(jnp.float32)
        prod = (xf * gw_ref[...].astype(jnp.float32).reshape(1, D)).astype(jnp.bfloat16).astype(jnp.float32)
        s = jnp.sum(prod, axis=-1, keepdims=True).astype(jnp.bfloat16).astype(jnp.float32)
        gate = jax.nn.sigmoid(s).astype(jnp.bfloat16).astype(jnp.float32)
        omg = (1.0 - gate).astype(jnp.bfloat16).astype(jnp.float32)
        dsk = dsk_ref[...].astype(jnp.float32).reshape(1, D)

        @pl.when(i > 0)
        def _():
            for n in range(NO):
                o_copy(i - 1, n).wait()

        for n in range(NO):
            cs = slice(n * OC, (n + 1) * OC)
            y = _nt_dot(h, ccat_ref[cs, :])
            b = acc_ref[:, cs].astype(jnp.bfloat16).astype(jnp.float32)
            skip = (xf[:, cs] * dsk[:, cs]).astype(jnp.bfloat16).astype(jnp.float32)
            t2 = (omg * b).astype(jnp.bfloat16).astype(jnp.float32)
            obuf[:, cs] = gate * (y + skip) + t2
            o_copy(i, n).start()

        @pl.when(i == nsteps - 1)
        def _():
            for n in range(NO):
                o_copy(i, n).wait()


@jax.jit
def pallas_gated_mix__ssm_conv_s5__glu_gated_geglu__prompt_kernel(
    A_x: jax.Array,
    A_Lambda_re: jax.Array,
    A_Lambda_im: jax.Array,
    A_B_re: jax.Array,
    A_B_im: jax.Array,
    A_C_re: jax.Array,
    A_C_im: jax.Array,
    A_log_dt: jax.Array,
    A_Dskip: jax.Array,
    B_x: jax.Array,
    B_w_gate: jax.Array,
    B_w_up: jax.Array,
    B_w_down: jax.Array,
    gate_w: jax.Array,
):
    Bsz, L, D = A_x.shape
    P = A_Lambda_re.shape[0]
    F = B_w_gate.shape[1]
    assert Bsz == 1
    T = T_BLK
    NF = F // F_BLK
    x2 = A_x.reshape(L, D)
    row = lambda a: a.reshape(1, -1)

    const = lambda shape: pl.BlockSpec(shape, lambda i: (0,))
    hbm = pl.BlockSpec(memory_space=pl.ANY)
    in_specs = [
        hbm,
        const((P,)), const((P,)), const((P,)), const((D,)), const((D,)),
        hbm, hbm, hbm, hbm, hbm, hbm, hbm,
    ]
    bf = jnp.bfloat16
    out = pl.pallas_call(
        functools.partial(_kernel, P=P, D=D, F=F, T=T),
        grid=(L // T,),
        in_specs=in_specs,
        out_specs=hbm,
        out_shape=jax.ShapeDtypeStruct((L, D), jnp.float32),
        scratch_shapes=[
            pltpu.VMEM((D, F), bf), pltpu.VMEM((D, F), bf), pltpu.VMEM((F, D), bf),
            pltpu.VMEM((2 * P, D), bf),
            pltpu.VMEM((D, 2 * P), bf),
            pltpu.VMEM((2 * P // 128, T, 128), jnp.float32),
            pltpu.VMEM((2 * P // 128, T, 128), bf),
            pltpu.VMEM((P // 128, 10, 8, 128), jnp.float32),
            pltpu.VMEM((P // 128, 8, 128), jnp.float32),
            pltpu.VMEM((T, D), jnp.float32),
            pltpu.VMEM((2, T, D), bf),
            pltpu.VMEM((T, D), jnp.float32),
            pltpu.SemaphoreType.DMA((4 + 3 * NF,)),
            pltpu.SemaphoreType.DMA((2,)),
            pltpu.SemaphoreType.DMA((4,)),
        ],
        compiler_params=pltpu.CompilerParams(
            dimension_semantics=("arbitrary",),
            vmem_limit_bytes=100 * 1024 * 1024,
        ),
    )(x2, A_Lambda_re, A_Lambda_im, A_log_dt, A_Dskip, gate_w,
      A_B_re, A_B_im, A_C_re, A_C_im, B_w_gate, B_w_up, B_w_down)
    return out.reshape(Bsz, L, D)
```

```python
import functools

import jax
import jax.numpy as jnp
import jax.experimental.pallas as pl
import jax.experimental.pallas.tpu as pltpu

T_BLK = 512
F_BLK = 512
N_A = 3


def _nt_dot(a, b):
    return jax.lax.dot_general(a, b, (((1,), (1,)), ((), ())),
                               preferred_element_type=jnp.float32)


def _cmul(ar, ai, br, bi):
    return ar * br - ai * bi, ar * bi + ai * br


def _bf(a):
    return a.astype(jnp.bfloat16).astype(jnp.float32)


def _tie(val, dep):
    d = dep[0:val.shape[0], 0:val.shape[1]]
    return jnp.where(d > jnp.inf, d, val)


def _kernel(x_hbm, lre_ref, lim_ref, ldt_ref, dsk_ref, gw_ref,
            bre_hbm, bim_hbm, cre_hbm, cim_hbm, wg_hbm, wu_hbm, wd_hbm,
            o_hbm,
            wg_v, wu_v, wd_v,
            bcat_ref, ccat_ref, v_ref, h_ref, tab_ref, carry_ref, acc_ref, gate_ref,
            xbuf, obuf, sems, xsem, osem,
            *, P, D, F, T):
    i = pl.program_id(0)
    NF = F // F_BLK
    HT = P // 128
    first = i == 0
    nsteps = pl.num_programs(0)
    slot = i % 2
    NO = 4
    OC = D // NO
    QT = T // 16

    def x_copy(step, sl):
        return pltpu.make_async_copy(
            x_hbm.at[pl.ds(pl.multiple_of(step * T, T), T), :], xbuf.at[sl], xsem.at[sl])

    def o_copy(step, n):
        return pltpu.make_async_copy(
            obuf.at[:, n * OC:(n + 1) * OC],
            o_hbm.at[pl.ds(pl.multiple_of(step * T, T), T), n * OC:(n + 1) * OC],
            osem.at[n])

    def g_copies(f):
        fs = pl.ds(pl.multiple_of(f * F_BLK, F_BLK), F_BLK)
        return [
            pltpu.make_async_copy(wg_hbm.at[:, fs], wg_v.at[:, fs], sems.at[4 + 3 * f]),
            pltpu.make_async_copy(wu_hbm.at[:, fs], wu_v.at[:, fs], sems.at[5 + 3 * f]),
            pltpu.make_async_copy(wd_hbm.at[fs, :], wd_v.at[fs, :], sems.at[6 + 3 * f]),
        ]

    def b_copies():
        return [pltpu.make_async_copy(bre_hbm, bcat_ref.at[0:P, :], sems.at[0]),
                pltpu.make_async_copy(bim_hbm, bcat_ref.at[P:2 * P, :], sems.at[1])]

    def c_copies():
        return [pltpu.make_async_copy(cre_hbm, ccat_ref.at[:, 0:P], sems.at[2]),
                pltpu.make_async_copy(cim_hbm, ccat_ref.at[:, P:2 * P], sems.at[3])]

    @pl.when(first)
    def _():
        x_copy(0, 0).start()
        g_copies(0)[0].start()
        lre = lre_ref[...].astype(jnp.float32).reshape(1, P)
        lim = lim_ref[...].astype(jnp.float32).reshape(1, P)
        dt = _bf(jnp.exp(ldt_ref[...].astype(jnp.float32).reshape(1, P)))
        mag = jnp.exp(dt * lre)
        a_re = mag * jnp.cos(dt * lim)
        a_im = mag * jnp.sin(dt * lim)
        nr = a_re - 1.0
        ni = a_im
        den = lre * lre + lim * lim
        m_re = (nr * lre + ni * lim) / den
        m_im = (ni * lre - nr * lim) / den
        a_im = -a_im
        pw = [(a_re, a_im)]
        for _ in range(7):
            pw.append(_cmul(pw[-1][0], pw[-1][1], a_re, a_im))
        rid = jax.lax.broadcasted_iota(jnp.int32, (8, P), 0)
        tabs = []
        for k in (1, 2, 4):
            tabs.append(jnp.where(rid >= k, pw[k - 1][0], 0.0))
            tabs.append(jnp.where(rid >= k, pw[k - 1][1], 0.0))
        tabs.append(jnp.concatenate([p[0] for p in pw], axis=0))
        tabs.append(jnp.concatenate([p[1] for p in pw], axis=0))
        tabs.append(jnp.broadcast_to(2.0 * m_re, (8, P)))
        tabs.append(jnp.broadcast_to(-2.0 * m_im, (8, P)))
        tabs.append(jnp.broadcast_to(-2.0 * m_re, (8, P)))
        for k in range(HT):
            for n in range(11):
                tab_ref[k, n] = tabs[n][:, k * 128:(k + 1) * 128]
        carry_ref[...] = jnp.zeros(carry_ref.shape, jnp.float32)
        acc_ref[...] = jnp.zeros(acc_ref.shape, jnp.float32)

    x_copy(i, slot).wait()
    x_ref = xbuf.at[slot]

    def dma_ctl(f):
        @pl.when(first)
        def _():
            for cp in g_copies(f):
                cp.wait()

            @pl.when(f + 1 < NF)
            def _():
                for cp in g_copies(f + 1):
                    cp.start()

            @pl.when(f == N_A - 1)
            def _():
                for cp in c_copies():
                    cp.start()

    def act(g, u):
        return (jax.nn.gelu(_bf(g), approximate=True) * _bf(u)).astype(jnp.bfloat16)

    def loop_a(f, carry):
        dma_ctl(f)
        fs = pl.ds(pl.multiple_of(f * F_BLK, F_BLK), F_BLK)
        xx = x_ref[...]
        g = jnp.dot(xx, wg_v[:, fs], preferred_element_type=jnp.float32)
        u = jnp.dot(xx, wu_v[:, fs], preferred_element_type=jnp.float32)
        acc_ref[...] += jnp.dot(act(g, u), wd_v[fs, :], preferred_element_type=jnp.float32)
        return carry

    def scan_q(k, q, st):
        tabs, c_re, c_im = st
        outs = []
        for half in range(2):
            r0 = q * 16 + half * 8
            v_re = v_ref[k, r0:r0 + 8, :]
            v_im = v_ref[HT + k, r0:r0 + 8, :]
            h_re = tabs[8] * v_re + tabs[9] * v_im
            h_im = tabs[10] * v_im + tabs[9] * v_re
            for n, sh in enumerate((1, 2, 4)):
                r_re = pltpu.roll(h_re, sh, 0)
                r_im = pltpu.roll(h_im, sh, 0)
                d_re, d_im = _cmul(tabs[2 * n], tabs[2 * n + 1], r_re, r_im)
                h_re = h_re + d_re
                h_im = h_im + d_im
            cb_re = jnp.broadcast_to(c_re, (8, 128))
            cb_im = jnp.broadcast_to(c_im, (8, 128))
            d_re, d_im = _cmul(tabs[6], tabs[7], cb_re, cb_im)
            h_re = h_re + d_re
            h_im = h_im + d_im
            c_re = h_re[7:8]
            c_im = h_im[7:8]
            outs.append((h_re, h_im))
        h_ref[k, q * 16:(q + 1) * 16, :] = jnp.concatenate(
            [outs[0][0], outs[1][0]], axis=0).astype(jnp.bfloat16)
        h_ref[HT + k, q * 16:(q + 1) * 16, :] = jnp.concatenate(
            [outs[0][1], outs[1][1]], axis=0).astype(jnp.bfloat16)
        return tabs, c_re, c_im

    TPI = HT // (NF - N_A)
    NG = F_BLK // 128
    NPIECE = 2 * NG + D // 128
    QTOT = TPI * QT

    def loop_b(f, carry):
        dma_ctl(f)
        k0 = (f - N_A) * TPI
        state = [None]

        def scan_piece(p, dep):
            for gq in range(p * QTOT // NPIECE, (p + 1) * QTOT // NPIECE):
                t, q = divmod(gq, QT)
                k = k0 + t
                if q == 0:
                    state[0] = ([tab_ref[k, n] for n in range(11)],
                                carry_ref[k, 0:1, :], carry_ref[k, 1:2, :])
                if dep is not None:
                    tabs, c_re, c_im = state[0]
                    state[0] = (tabs, _tie(c_re, dep), c_im)
                    dep = None
                state[0] = scan_q(k, q, state[0])
                if q == QT - 1:
                    carry_ref[k, 0:1, :] = state[0][1]
                    carry_ref[k, 1:2, :] = state[0][2]

        xx = x_ref[...]
        p = 0
        dep = None
        hms = []
        for n in range(NG):
            fs = pl.ds(pl.multiple_of(f * F_BLK + n * 128, 128), 128)
            scan_piece(p, dep); p += 1
            g = jnp.dot(xx, wg_v[:, fs], preferred_element_type=jnp.float32)
            scan_piece(p, g); p += 1
            u = jnp.dot(xx, wu_v[:, fs], preferred_element_type=jnp.float32)
            dep = u
            hms.append(act(g, u))
        hm = jnp.concatenate(hms, axis=1)
        fs = pl.ds(pl.multiple_of(f * F_BLK, F_BLK), F_BLK)
        for n in range(D // 128):
            scan_piece(p, dep); p += 1
            cs = slice(n * 128, (n + 1) * 128)
            d = jnp.dot(hm, wd_v[fs, cs], preferred_element_type=jnp.float32)
            dep = d
            acc_ref[:, cs] += d
        return carry

    @pl.when(first)
    def _():
        cg, cu, cd = g_copies(0)
        cg.wait()
        cu.start()
        cd.start()
        xx = x_ref[...]
        g = jnp.dot(xx, wg_v[:, 0:F_BLK], preferred_element_type=jnp.float32)
        cu.wait()
        cd.wait()
        for cp in g_copies(1) + b_copies():
            cp.start()
        u = jnp.dot(xx, wu_v[:, 0:F_BLK], preferred_element_type=jnp.float32)
        acc_ref[...] += jnp.dot(act(g, u), wd_v[0:F_BLK, :], preferred_element_type=jnp.float32)

    jax.lax.fori_loop(jnp.where(first, 1, 0), N_A, loop_a, 0)

    @pl.when(first)
    def _():
        for cp in b_copies():
            cp.wait()

    NB = 4
    x = x_ref[...]
    gw = gw_ref[...].astype(jnp.float32).reshape(1, D)
    RB = T // NB
    for n in range(NB):
        w = 2 * P // NB
        v = _nt_dot(x, bcat_ref[n * w:(n + 1) * w, :])
        for k in range(w // 128):
            v_ref[n * (w // 128) + k] = v[:, k * 128:(k + 1) * 128]
        gwt = jnp.concatenate([_tie(gw[:, 0:128], v), gw[:, 128:]], axis=1)
        xf = x_ref[n * RB:(n + 1) * RB, :].astype(jnp.float32)
        s = jnp.sum(_bf(xf * gwt), axis=-1, keepdims=True)
        gate_ref[n * RB:(n + 1) * RB, :] = jnp.broadcast_to(
            _bf(jax.nn.sigmoid(_bf(s))), (RB, 128))

    jax.lax.fori_loop(N_A, NF, loop_b, 0)

    @pl.when(first)
    def _():
        for cp in c_copies():
            cp.wait()

    @pl.when(i + 1 < nsteps)
    def _():
        x_copy(i + 1, 1 - slot).start()

    @pl.when(i > 0)
    def _():
        for n in range(NO):
            o_copy(i - 1, n).wait()

    h = jnp.concatenate([h_ref[k] for k in range(2 * HT)], axis=1)
    gate = gate_ref[:, 0:1]
    omg = _bf(1.0 - gate)
    dsk = dsk_ref[...].astype(jnp.float32).reshape(1, D)
    for n in range(NO):
        cs = slice(n * OC, (n + 1) * OC)
        y = _nt_dot(h, ccat_ref[cs, :])
        b = _bf(acc_ref[:, cs])
        acc_ref[:, cs] = jnp.zeros((T, OC), jnp.float32)
        skip = _bf(x_ref[:, cs].astype(jnp.float32) * dsk[:, cs])
        obuf[:, cs] = gate * (y + skip) + _bf(omg * b)
        o_copy(i, n).start()

    @pl.when(i == nsteps - 1)
    def _():
        for n in range(NO):
            o_copy(i, n).wait()


@jax.jit
def pallas_gated_mix__ssm_conv_s5__glu_gated_geglu__prompt_kernel(
    A_x: jax.Array,
    A_Lambda_re: jax.Array,
    A_Lambda_im: jax.Array,
    A_B_re: jax.Array,
    A_B_im: jax.Array,
    A_C_re: jax.Array,
    A_C_im: jax.Array,
    A_log_dt: jax.Array,
    A_Dskip: jax.Array,
    B_x: jax.Array,
    B_w_gate: jax.Array,
    B_w_up: jax.Array,
    B_w_down: jax.Array,
    gate_w: jax.Array,
):
    Bsz, L, D = A_x.shape
    P = A_Lambda_re.shape[0]
    F = B_w_gate.shape[1]
    assert Bsz == 1
    T = T_BLK
    NF = F // F_BLK
    x2 = A_x.reshape(L, D)

    const = lambda shape: pl.BlockSpec(shape, lambda i: (0,))
    hbm = pl.BlockSpec(memory_space=pl.ANY)
    in_specs = [
        hbm,
        const((P,)), const((P,)), const((P,)), const((D,)), const((D,)),
        hbm, hbm, hbm, hbm, hbm, hbm, hbm,
    ]
    bf = jnp.bfloat16
    out = pl.pallas_call(
        functools.partial(_kernel, P=P, D=D, F=F, T=T),
        grid=(L // T,),
        in_specs=in_specs,
        out_specs=hbm,
        out_shape=jax.ShapeDtypeStruct((L, D), jnp.float32),
        scratch_shapes=[
            pltpu.VMEM((D, F), bf), pltpu.VMEM((D, F), bf), pltpu.VMEM((F, D), bf),
            pltpu.VMEM((2 * P, D), bf),
            pltpu.VMEM((D, 2 * P), bf),
            pltpu.VMEM((2 * P // 128, T, 128), jnp.float32),
            pltpu.VMEM((2 * P // 128, T, 128), bf),
            pltpu.VMEM((P // 128, 11, 8, 128), jnp.float32),
            pltpu.VMEM((P // 128, 8, 128), jnp.float32),
            pltpu.VMEM((T, D), jnp.float32),
            pltpu.VMEM((T, 128), jnp.float32),
            pltpu.VMEM((2, T, D), bf),
            pltpu.VMEM((T, D), jnp.float32),
            pltpu.SemaphoreType.DMA((4 + 3 * NF,)),
            pltpu.SemaphoreType.DMA((2,)),
            pltpu.SemaphoreType.DMA((4,)),
        ],
        compiler_params=pltpu.CompilerParams(
            dimension_semantics=("arbitrary",),
            vmem_limit_bytes=100 * 1024 * 1024,
        ),
    )(x2, A_Lambda_re, A_Lambda_im, A_log_dt, A_Dskip, gate_w,
      A_B_re, A_B_im, A_C_re, A_C_im, B_w_gate, B_w_up, B_w_down)
    return out.reshape(Bsz, L, D)
```

```python
import functools

import jax
import jax.numpy as jnp
import jax.experimental.pallas as pl
import jax.experimental.pallas.tpu as pltpu

T_BLK = 512
F_BLK = 512
N_A = 3


def _nt_dot(a, b):
    return jax.lax.dot_general(a, b, (((1,), (1,)), ((), ())),
                               preferred_element_type=jnp.float32)


def _cmul(ar, ai, br, bi):
    return ar * br - ai * bi, ar * bi + ai * br


def _bf(a):
    return a.astype(jnp.bfloat16).astype(jnp.float32)


def _tie(val, dep):
    d = dep[0:val.shape[0], 0:val.shape[1]]
    return jnp.where(d > jnp.inf, d, val)


def _kernel(x_hbm, lre_ref, lim_ref, ldt_ref, dsk_ref, gw_ref,
            bre_hbm, bim_hbm, cre_hbm, cim_hbm, wg_hbm, wu_hbm, wd_hbm,
            o_hbm,
            wg_v, wu_v, wd_v,
            bcat_ref, ccat_ref, v_ref, h_ref, tab_ref, carry_ref, acc_ref, gate_ref,
            xbuf, obuf, sems, xsem, osem,
            *, P, D, F, T):
    i = pl.program_id(0)
    NF = F // F_BLK
    HT = P // 128
    first = i == 0
    nsteps = pl.num_programs(0)
    slot = i % 2
    NO = 8
    OC = D // NO
    QT = T // 16

    def x_copy(step, sl):
        return pltpu.make_async_copy(
            x_hbm.at[pl.ds(pl.multiple_of(step * T, T), T), :], xbuf.at[sl], xsem.at[sl])

    def o_copy(step, n):
        return pltpu.make_async_copy(
            obuf.at[:, n * OC:(n + 1) * OC],
            o_hbm.at[pl.ds(pl.multiple_of(step * T, T), T), n * OC:(n + 1) * OC],
            osem.at[n])

    def g_copy(f, which):
        fs = pl.ds(pl.multiple_of(f * F_BLK, F_BLK), F_BLK)
        if which == 0:
            return pltpu.make_async_copy(wg_hbm.at[:, fs], wg_v.at[:, fs], sems.at[4 + 3 * f])
        if which == 1:
            return pltpu.make_async_copy(wu_hbm.at[:, fs], wu_v.at[:, fs], sems.at[5 + 3 * f])
        return pltpu.make_async_copy(wd_hbm.at[fs, :], wd_v.at[fs, :], sems.at[6 + 3 * f])

    def g_copies(f):
        return [g_copy(f, 0), g_copy(f, 1), g_copy(f, 2)]

    def b_copies():
        return [pltpu.make_async_copy(bre_hbm, bcat_ref.at[0:P, :], sems.at[0]),
                pltpu.make_async_copy(bim_hbm, bcat_ref.at[P:2 * P, :], sems.at[1])]

    def c_copies():
        return [pltpu.make_async_copy(cre_hbm, ccat_ref.at[:, 0:P], sems.at[2]),
                pltpu.make_async_copy(cim_hbm, ccat_ref.at[:, P:2 * P], sems.at[3])]

    @pl.when(first)
    def _():
        x_copy(0, 0).start()
        g_copy(0, 0).start()
        lre = lre_ref[...].astype(jnp.float32).reshape(1, P)
        lim = lim_ref[...].astype(jnp.float32).reshape(1, P)
        dt = _bf(jnp.exp(ldt_ref[...].astype(jnp.float32).reshape(1, P)))
        mag = jnp.exp(dt * lre)
        a_re = mag * jnp.cos(dt * lim)
        a_im = mag * jnp.sin(dt * lim)
        nr = a_re - 1.0
        ni = a_im
        den = lre * lre + lim * lim
        m_re = (nr * lre + ni * lim) / den
        m_im = (ni * lre - nr * lim) / den
        a_im = -a_im
        pw = [(a_re, a_im)]
        for _ in range(7):
            pw.append(_cmul(pw[-1][0], pw[-1][1], a_re, a_im))
        rid = jax.lax.broadcasted_iota(jnp.int32, (8, P), 0)
        tabs = []
        for k in (1, 2, 4):
            tabs.append(jnp.where(rid >= k, pw[k - 1][0], 0.0))
            tabs.append(jnp.where(rid >= k, pw[k - 1][1], 0.0))
        tabs.append(jnp.concatenate([p[0] for p in pw], axis=0))
        tabs.append(jnp.concatenate([p[1] for p in pw], axis=0))
        tabs.append(jnp.broadcast_to(2.0 * m_re, (8, P)))
        tabs.append(jnp.broadcast_to(-2.0 * m_im, (8, P)))
        tabs.append(jnp.broadcast_to(-2.0 * m_re, (8, P)))
        for k in range(HT):
            for n in range(11):
                tab_ref[k, n] = tabs[n][:, k * 128:(k + 1) * 128]
        carry_ref[...] = jnp.zeros(carry_ref.shape, jnp.float32)
        acc_ref[...] = jnp.zeros(acc_ref.shape, jnp.float32)

    x_copy(i, slot).wait()
    x_ref = xbuf.at[slot]

    def dma_ctl(f):
        @pl.when(first)
        def _():
            for cp in g_copies(f):
                cp.wait()

            @pl.when(f + 1 < NF)
            def _():
                for cp in g_copies(f + 1):
                    cp.start()

            @pl.when(f == N_A - 1)
            def _():
                for cp in c_copies():
                    cp.start()

    def act(g, u):
        return (jax.nn.gelu(_bf(g), approximate=True) * _bf(u)).astype(jnp.bfloat16)

    def loop_a(f, carry):
        dma_ctl(f)
        fs = pl.ds(pl.multiple_of(f * F_BLK, F_BLK), F_BLK)
        xx = x_ref[...]
        g = jnp.dot(xx, wg_v[:, fs], preferred_element_type=jnp.float32)
        u = jnp.dot(xx, wu_v[:, fs], preferred_element_type=jnp.float32)
        acc_ref[...] += jnp.dot(act(g, u), wd_v[fs, :], preferred_element_type=jnp.float32)
        return carry

    def scan_q(k, q, st):
        tabs, c_re, c_im = st
        outs = []
        for half in range(2):
            r0 = q * 16 + half * 8
            v_re = v_ref[k, r0:r0 + 8, :]
            v_im = v_ref[HT + k, r0:r0 + 8, :]
            h_re = tabs[8] * v_re + tabs[9] * v_im
            h_im = tabs[10] * v_im + tabs[9] * v_re
            for n, sh in enumerate((1, 2, 4)):
                r_re = pltpu.roll(h_re, sh, 0)
                r_im = pltpu.roll(h_im, sh, 0)
                d_re, d_im = _cmul(tabs[2 * n], tabs[2 * n + 1], r_re, r_im)
                h_re = h_re + d_re
                h_im = h_im + d_im
            cb_re = jnp.broadcast_to(c_re, (8, 128))
            cb_im = jnp.broadcast_to(c_im, (8, 128))
            d_re, d_im = _cmul(tabs[6], tabs[7], cb_re, cb_im)
            h_re = h_re + d_re
            h_im = h_im + d_im
            c_re = h_re[7:8]
            c_im = h_im[7:8]
            outs.append((h_re, h_im))
        h_ref[k, q * 16:(q + 1) * 16, :] = jnp.concatenate(
            [outs[0][0], outs[1][0]], axis=0).astype(jnp.bfloat16)
        h_ref[HT + k, q * 16:(q + 1) * 16, :] = jnp.concatenate(
            [outs[0][1], outs[1][1]], axis=0).astype(jnp.bfloat16)
        return tabs, c_re, c_im

    TPI = HT // (NF - N_A)
    NG = F_BLK // 128
    NPIECE = 2 * NG + D // 128
    QTOT = TPI * QT

    def loop_b(f, carry):
        dma_ctl(f)
        k0 = (f - N_A) * TPI
        state = [None]

        def scan_piece(p, dep):
            for gq in range(p * QTOT // NPIECE, (p + 1) * QTOT // NPIECE):
                t, q = divmod(gq, QT)
                k = k0 + t
                if q == 0:
                    state[0] = ([tab_ref[k, n] for n in range(11)],
                                carry_ref[k, 0:1, :], carry_ref[k, 1:2, :])
                if dep is not None:
                    tabs, c_re, c_im = state[0]
                    state[0] = (tabs, _tie(c_re, dep), c_im)
                    dep = None
                state[0] = scan_q(k, q, state[0])
                if q == QT - 1:
                    carry_ref[k, 0:1, :] = state[0][1]
                    carry_ref[k, 1:2, :] = state[0][2]

        xx = x_ref[...]
        p = 0
        dep = None
        hms = []
        for n in range(NG):
            fs = pl.ds(pl.multiple_of(f * F_BLK + n * 128, 128), 128)
            scan_piece(p, dep); p += 1
            g = jnp.dot(xx, wg_v[:, fs], preferred_element_type=jnp.float32)
            scan_piece(p, g); p += 1
            u = jnp.dot(xx, wu_v[:, fs], preferred_element_type=jnp.float32)
            dep = u
            hms.append(act(g, u))
        hm = jnp.concatenate(hms, axis=1)
        fs = pl.ds(pl.multiple_of(f * F_BLK, F_BLK), F_BLK)
        for n in range(D // 128):
            scan_piece(p, dep); p += 1
            cs = slice(n * 128, (n + 1) * 128)
            d = jnp.dot(hm, wd_v[fs, cs], preferred_element_type=jnp.float32)
            dep = d
            acc_ref[:, cs] += d
        return carry

    @pl.when(first)
    def _():
        cg, cu, cd = g_copies(0)
        cg.wait()
        cu.start()
        cd.start()
        xx = x_ref[...]
        g = jnp.dot(xx, wg_v[:, 0:F_BLK], preferred_element_type=jnp.float32)
        cu.wait()
        cd.wait()
        for cp in g_copies(1) + b_copies():
            cp.start()
        u = jnp.dot(xx, wu_v[:, 0:F_BLK], preferred_element_type=jnp.float32)
        acc_ref[...] += jnp.dot(act(g, u), wd_v[0:F_BLK, :], preferred_element_type=jnp.float32)

    jax.lax.fori_loop(jnp.where(first, 1, 0), N_A, loop_a, 0)

    @pl.when(first)
    def _():
        for cp in b_copies():
            cp.wait()

    NB = 16
    x = x_ref[...]
    gw = gw_ref[...].astype(jnp.float32).reshape(1, D)
    RB = T // NB
    for n in range(NB):
        w = 2 * P // NB
        v = _nt_dot(x, bcat_ref[n * w:(n + 1) * w, :])
        for k in range(w // 128):
            v_ref[n * (w // 128) + k] = v[:, k * 128:(k + 1) * 128]
        gwt = jnp.concatenate([_tie(gw[:, 0:128], v), gw[:, 128:]], axis=1)
        xf = x_ref[n * RB:(n + 1) * RB, :].astype(jnp.float32)
        s = jnp.sum(_bf(xf * gwt), axis=-1, keepdims=True)
        gate_ref[n * RB:(n + 1) * RB, :] = jnp.broadcast_to(
            _bf(jax.nn.sigmoid(_bf(s))), (RB, 128))

    jax.lax.fori_loop(N_A, NF, loop_b, 0)

    @pl.when(first)
    def _():
        for cp in c_copies():
            cp.wait()

    @pl.when(i + 1 < nsteps)
    def _():
        x_copy(i + 1, 1 - slot).start()

    @pl.when(i > 0)
    def _():
        for n in range(NO):
            o_copy(i - 1, n).wait()

    h = jnp.concatenate([h_ref[k] for k in range(2 * HT)], axis=1)
    gate = gate_ref[:, 0:1]
    omg = _bf(1.0 - gate)
    dsk = dsk_ref[...].astype(jnp.float32).reshape(1, D)
    for n in range(NO):
        cs = slice(n * OC, (n + 1) * OC)
        y = _nt_dot(h, ccat_ref[cs, :])
        b = _bf(acc_ref[:, cs])
        acc_ref[:, cs] = jnp.zeros((T, OC), jnp.float32)
        skip = _bf(x_ref[:, cs].astype(jnp.float32) * dsk[:, cs])
        obuf[:, cs] = gate * (y + skip) + _bf(omg * b)
        o_copy(i, n).start()

    @pl.when(i == nsteps - 1)
    def _():
        for n in range(NO):
            o_copy(i, n).wait()


@jax.jit
def pallas_gated_mix__ssm_conv_s5__glu_gated_geglu__prompt_kernel(
    A_x: jax.Array,
    A_Lambda_re: jax.Array,
    A_Lambda_im: jax.Array,
    A_B_re: jax.Array,
    A_B_im: jax.Array,
    A_C_re: jax.Array,
    A_C_im: jax.Array,
    A_log_dt: jax.Array,
    A_Dskip: jax.Array,
    B_x: jax.Array,
    B_w_gate: jax.Array,
    B_w_up: jax.Array,
    B_w_down: jax.Array,
    gate_w: jax.Array,
):
    Bsz, L, D = A_x.shape
    P = A_Lambda_re.shape[0]
    F = B_w_gate.shape[1]
    assert Bsz == 1
    T = T_BLK
    NF = F // F_BLK
    x2 = A_x.reshape(L, D)

    const = lambda shape: pl.BlockSpec(shape, lambda i: (0,))
    hbm = pl.BlockSpec(memory_space=pl.ANY)
    in_specs = [
        hbm,
        const((P,)), const((P,)), const((P,)), const((D,)), const((D,)),
        hbm, hbm, hbm, hbm, hbm, hbm, hbm,
    ]
    bf = jnp.bfloat16
    out = pl.pallas_call(
        functools.partial(_kernel, P=P, D=D, F=F, T=T),
        grid=(L // T,),
        in_specs=in_specs,
        out_specs=hbm,
        out_shape=jax.ShapeDtypeStruct((L, D), jnp.float32),
        scratch_shapes=[
            pltpu.VMEM((D, F), bf), pltpu.VMEM((D, F), bf), pltpu.VMEM((F, D), bf),
            pltpu.VMEM((2 * P, D), bf),
            pltpu.VMEM((D, 2 * P), bf),
            pltpu.VMEM((2 * P // 128, T, 128), jnp.float32),
            pltpu.VMEM((2 * P // 128, T, 128), bf),
            pltpu.VMEM((P // 128, 11, 8, 128), jnp.float32),
            pltpu.VMEM((P // 128, 8, 128), jnp.float32),
            pltpu.VMEM((T, D), jnp.float32),
            pltpu.VMEM((T, 128), jnp.float32),
            pltpu.VMEM((2, T, D), bf),
            pltpu.VMEM((T, D), jnp.float32),
            pltpu.SemaphoreType.DMA((4 + 3 * NF,)),
            pltpu.SemaphoreType.DMA((2,)),
            pltpu.SemaphoreType.DMA((8,)),
        ],
        compiler_params=pltpu.CompilerParams(
            dimension_semantics=("arbitrary",),
            vmem_limit_bytes=100 * 1024 * 1024,
        ),
    )(x2, A_Lambda_re, A_Lambda_im, A_log_dt, A_Dskip, gate_w,
      A_B_re, A_B_im, A_C_re, A_C_im, B_w_gate, B_w_up, B_w_down)
    return out.reshape(Bsz, L, D)
```
